```python
import os as _os
_os.environ.setdefault("JAX_PLATFORMS", "cpu")
import jax
import jax.numpy as jnp

def _softmax(x, axis=-1):
    return jax.nn.softmax(x, axis=axis)
def _gelu(x):
    return jax.nn.gelu(x, approximate=True)
def _silu(x):
    return jax.nn.silu(x)
def _sigmoid(x):
    return jax.nn.sigmoid(x)
def _layernorm(x, axis=-1, eps=1e-5):
    m = jnp.mean(x, axis=axis, keepdims=True)
    v = jnp.var(x, axis=axis, keepdims=True)
    return (x - m) / jnp.sqrt(v + eps)
def _scatter_add(tgt, idx, src, axis=0):
    return tgt.at[idx].add(src)
def _segment_sum(src, seg, n):
    return jax.ops.segment_sum(src, seg, n)
class _Rng:
    def __init__(self, key):
        self._k = key
    def _next(self):
        self._k, sub = jax.random.split(self._k)
        return sub
    def normal(self, shape):
        return jax.random.normal(self._next(), shape, dtype=jnp.bfloat16)
    def randint(self, lo, hi, shape):
        return jax.random.randint(self._next(), shape, lo, hi, dtype=jnp.int32)
    def uniform(self, shape, lo=0.0, hi=1.0):
        return jax.random.uniform(self._next(), shape, jnp.bfloat16, lo, hi)
    def permutation(self, n):
        return jax.random.permutation(self._next(), n)


kernel_name = 'sequential_preLN__mha_block__swiglu_ffn__prompt'

def setup_inputs():
    _rng = _Rng(jax.random.key(int.from_bytes(__import__("os").urandom(4), "little")))
    _w = (lambda a: (lambda t: t.astype(jnp.bfloat16) if jnp.issubdtype(t.dtype, jnp.floating) else t)(jnp.asarray(a)))
    def _A_setup():
        B, S, D, H = 1, 2048, 640, 32
        return {
            "x": _w((lambda *s: _rng.normal(s) * 0.05)(B, S, D)),
            "wqkv": _w((lambda *s: _rng.normal(s) * 0.05)(D, 3 * D)),
            "wo": _w((lambda *s: _rng.normal(s) * 0.05)(D, D)),
        }
    _A_in = _A_setup()

    def _B_setup():
        B, S, D, F = 1, 2048, 640, 1728
        return {
            "x": _w((lambda *s: _rng.normal(s) * 0.05)(B, S, D)),
            "w_gate": _w((lambda *s: _rng.normal(s) * 0.05)(D, F)),
            "w_up": _w((lambda *s: _rng.normal(s) * 0.05)(D, F)),
            "w_down": _w((lambda *s: _rng.normal(s) * 0.05)(F, D)),
        }
    _B_in = _B_setup()

    return {
        "A_x": _A_in["x"],
        "A_wqkv": _A_in["wqkv"],
        "A_wo": _A_in["wo"],
        "B_x": _B_in["x"],
        "B_w_gate": _B_in["w_gate"],
        "B_w_up": _B_in["w_up"],
        "B_w_down": _B_in["w_down"],
    }

def reference(A_x, A_wqkv, A_wo, B_x, B_w_gate, B_w_up, B_w_down):
    def _A_ref(x, wqkv, wo):
        B, S, D = x.shape
        H = 32
        Dh = D // H
        qkv = (lambda x, *d: x.transpose(*d))((x @ wqkv).reshape(B, S, 3, H, Dh), 2, 0, 3, 1, 4)
        q, k, v = qkv[0], qkv[1], qkv[2]
        scores = jnp.einsum("bhqd,bhkd->bhqk", q, k) * (Dh ** -0.5)
        p = _softmax(scores, axis=-1)
        o = jnp.einsum("bhqk,bhkd->bhqd", p, v)
        return (lambda x, *d: x.transpose(*d))(o, 0, 2, 1, 3).reshape(B, S, D) @ wo

    def _B_ref(x, w_gate, w_up, w_down):
        g = _silu(x @ w_gate)
        u = x @ w_up
        return (g * u) @ w_down

    x = A_x
    h = x + _A_ref(_layernorm(x, axis=-1), A_wqkv, A_wo)
    h2 = h + _B_ref(_layernorm(h, axis=-1), B_w_gate, B_w_up, B_w_down)
    return h2
```

```python
import math

import jax
import jax.numpy as jnp
from jax import lax
import jax.experimental.pallas as pl
import jax.experimental.pallas.tpu as pltpu

_H = 32
_TQ = 512
_TK = 128
_VR = 24
_EPS = 1e-5
_NT_DIMS = (((1,), (1,)), ((), ()))
F32 = jnp.float32
BF16 = jnp.bfloat16


def _layernorm(x):
    m = jnp.mean(x, axis=-1, keepdims=True)
    d = x - m
    v = jnp.mean(d * d, axis=-1, keepdims=True)
    return d * lax.rsqrt(v + _EPS)


def _kernel(x_hbm, wqkv_hbm, wo_hbm, wg_hbm, wu_hbm, wd_hbm, out_ref,
            x_v, wqkv_v, wo_v, wg_v, wu_v, wd_v, sems,
            xn_v, k_v, qt_v, vt_v, qm_v, s0_v, s1_v, m_v, ot_v):
    S, D = x_v.shape
    Dh = D // _H
    NT = D // 128
    NQ = S // _TQ
    qb = pl.program_id(0)
    qscale = (Dh ** -0.5) * math.log2(math.e)

    copies = [pltpu.make_async_copy(s, d, sems.at[i]) for i, (s, d) in enumerate(
        [(x_hbm, x_v), (wqkv_hbm, wqkv_v), (wo_hbm, wo_v), (wg_hbm, wg_v),
         (wu_hbm, wu_v), (wd_hbm, wd_v)])]

    def head_q(t):
        h = t % _H
        b = t // _H
        f0 = h * Dh
        t0 = f0 // 128
        off = f0 % 128
        t1 = jnp.minimum(t0 + 1, NT - 1)
        r = lax.broadcasted_iota(jnp.int32, (128, _TQ), 0)
        lo = qt_v[b, pl.ds(pl.multiple_of(t0 * 128, 128), 128), :].astype(F32)
        hi = qt_v[b, pl.ds(pl.multiple_of(t1 * 128, 128), 128), :].astype(F32)
        q = jnp.where((r >= off) & (r < off + Dh), lo,
                      jnp.where(r < off + Dh - 128, hi, 0.0))
        kt = jnp.where(off + Dh > 128, NT + t0, t0)
        return q.astype(BF16), kt

    def stage(t, s_cur, s_nxt, m_cur, do_b=True):
        tn = jnp.minimum(t + 1, NQ * _H - 1)
        q, kt = head_q(tn)
        qm_v[...] = q
        m_nxt = jnp.full((8, _TQ), -jnp.inf, F32)
        if do_b:
            f0 = (t % _H) * Dh
            r0 = pl.multiple_of((f0 // 8) * 8, 8)
            r = lax.broadcasted_iota(jnp.int32, (_VR, 128), 0) - f0 % 8
            in_head = (r >= 0) & (r < Dh)
            acc = jnp.zeros((_VR, _TQ), F32)
        for c in range(S // _TK):
            sl = pl.ds(c * _TK, _TK)
            s = jnp.dot(k_v[kt, sl, :], qm_v[...], preferred_element_type=F32)
            s_nxt[sl, :] = s
            m_nxt = jnp.maximum(m_nxt, jnp.max(s.reshape(_TK // 8, 8, _TQ), axis=0))
            if do_b:
                p = jnp.exp2(s_cur[sl, :] - m_cur)
                v = jnp.where(in_head, vt_v[c, pl.ds(r0, _VR), :], 1.0)
                acc = acc + jnp.dot(v, p, preferred_element_type=F32)
        if do_b:
            rq = lax.broadcasted_iota(jnp.int32, (_VR, _TQ), 0) - f0 % 8
            hq = (rq >= 0) & (rq < Dh)
            l = jnp.max(jnp.where(hq, 0.0, acc), axis=0, keepdims=True)
            w = pl.ds(r0, _VR)
            ot_v[w, :] = jnp.where(hq, acc / l, ot_v[w, :])
        return jnp.max(m_nxt, axis=0, keepdims=True)

    @pl.when(qb == 0)
    def _():
        for cp in copies:
            cp.start()
        ot_v[...] = jnp.zeros_like(ot_v)
        copies[0].wait()

        def ln_body(i, carry):
            sl = pl.ds(pl.multiple_of(i * 256, 256), 256)
            xn_v[sl, :] = _layernorm(x_v[sl, :].astype(F32)).astype(BF16)
            return carry
        lax.fori_loop(0, S // 256, ln_body, 0)
        copies[1].wait()

        def proj_body(i, carry):
            sl = pl.ds(pl.multiple_of(i * _TQ, _TQ), _TQ)
            xn = xn_v[sl, :]
            q = jnp.dot(xn, wqkv_v[:, 0:D], preferred_element_type=F32) * qscale
            qt_v[i] = q.T.astype(BF16)
            k = jnp.dot(xn, wqkv_v[:, D:2 * D], preferred_element_type=F32)
            lane = lax.broadcasted_iota(jnp.int32, (_TQ, 128), 1)
            for j in range(NT):
                kj = k[:, j * 128:(j + 1) * 128]
                k_v[j, sl, :] = kj.astype(BF16)
                if j + 1 < NT:
                    kn = k[:, (j + 1) * 128:(j + 2) * 128]
                    k_v[NT + j, sl, :] = jnp.where(lane >= 64, kj, kn).astype(BF16)
            v = jnp.dot(xn, wqkv_v[:, 2 * D:3 * D], preferred_element_type=F32)
            vt = v.T
            for j in range(_TQ // _TK):
                vt_v[i * (_TQ // _TK) + j] = vt[:, j * _TK:(j + 1) * _TK]
            return carry
        lax.fori_loop(0, NQ, proj_body, 0)
        m_v[...] = stage(-1, None, s0_v, None, do_b=False)

    def attn_body(i, m):
        t = qb * _H + 2 * i
        m = stage(t, s0_v, s1_v, m)
        m = stage(t + 1, s1_v, s0_v, m)
        return m
    m_v[...] = lax.fori_loop(0, _H // 2, attn_body, m_v[...])

    @pl.when(qb == 0)
    def _():
        for cp in copies[2:]:
            cp.wait()

    TS = 256
    for j in range(_TQ // TS):
        o = ot_v[:, j * TS:(j + 1) * TS].T.astype(BF16)
        xs = x_v[pl.ds(pl.multiple_of(qb * _TQ + j * TS, TS), TS), :].astype(F32)
        h = xs + jnp.dot(o, wo_v[...], preferred_element_type=F32)
        hn = _layernorm(h).astype(BF16)
        g = lax.dot_general(hn, wg_v[...], _NT_DIMS, preferred_element_type=F32)
        u = lax.dot_general(hn, wu_v[...], _NT_DIMS, preferred_element_type=F32)
        a = (g * jax.nn.sigmoid(g) * u).astype(BF16)
        y = h + jnp.dot(a, wd_v[...], preferred_element_type=F32)
        out_ref[j * TS:(j + 1) * TS, :] = y.astype(out_ref.dtype)


@jax.jit
def pallas_sequential_preLN__mha_block__swiglu_ffn__prompt_kernel(
    A_x: jax.Array,
    A_wqkv: jax.Array,
    A_wo: jax.Array,
    B_x: jax.Array,
    B_w_gate: jax.Array,
    B_w_up: jax.Array,
    B_w_down: jax.Array,
):
    del B_x
    B, S, D = A_x.shape
    assert B == 1
    x = A_x.reshape(S, D)
    NT = D // 128
    ins = (x, A_wqkv, A_wo, B_w_gate.T, B_w_up.T, B_w_down)
    out = pl.pallas_call(
        _kernel,
        grid=(S // _TQ,),
        in_specs=[pl.BlockSpec(memory_space=pltpu.HBM)] * len(ins),
        out_specs=pl.BlockSpec((_TQ, D), lambda i: (i, 0)),
        out_shape=jax.ShapeDtypeStruct((S, D), A_x.dtype),
        scratch_shapes=[pltpu.VMEM(a.shape, a.dtype) for a in ins] + [
            pltpu.SemaphoreType.DMA((len(ins),)),
            pltpu.VMEM((S, D), BF16),
            pltpu.VMEM((2 * NT - 1, S, 128), BF16),
            pltpu.VMEM((S // _TQ, D, _TQ), BF16),
            pltpu.VMEM((S // _TK, D, _TK), F32),
            pltpu.VMEM((128, _TQ), BF16),
            pltpu.VMEM((S, _TQ), F32),
            pltpu.VMEM((S, _TQ), F32),
            pltpu.VMEM((1, _TQ), F32),
            pltpu.VMEM((D, _TQ), F32),
        ],
        compiler_params=pltpu.CompilerParams(
            dimension_semantics=("arbitrary",),
            vmem_limit_bytes=110 * 1024 * 1024),
        name="preln_mha_swiglu",
    )(*ins)
    return out.reshape(B, S, D)
```

```python
import math

import jax
import jax.numpy as jnp
from jax import lax
import jax.experimental.pallas as pl
import jax.experimental.pallas.tpu as pltpu

_H = 32
_TQ = 512
_TK = 128
_VR = 24
_UH = 8
_LAG = 3
_EPS = 1e-5
_NT_DIMS = (((1,), (1,)), ((), ()))
F32 = jnp.float32
BF16 = jnp.bfloat16


def _layernorm(x):
    m = jnp.mean(x, axis=-1, keepdims=True)
    d = x - m
    v = jnp.mean(d * d, axis=-1, keepdims=True)
    return d * lax.rsqrt(v + _EPS)


def _kernel(x_hbm, wqkv_hbm, wo_hbm, wg_hbm, wu_hbm, wd_hbm, out_ref,
            x_v, wqkv_v, wo_v, wgu_v, wd_v, sems,
            k_v, qm_v, vt_v, s_v, m_v, mr_v, ot_v):
    S, D = x_v.shape
    Dh = D // _H
    NT = D // 128
    NQ = S // _TQ
    qb = pl.program_id(0)
    qscale = (Dh ** -0.5) * math.log2(math.e)

    F = wd_v.shape[0]
    FM = F // 128 * 128
    FT = F - FM
    pairs = [
        (x_hbm.at[0:_TQ], x_v.at[0:_TQ]), (wqkv_hbm, wqkv_v),
        (x_hbm.at[_TQ:S], x_v.at[_TQ:S]), (wo_hbm, wo_v),
        (wg_hbm.at[0:FM], wgu_v.at[0:FM]), (wu_hbm.at[0:FM], wgu_v.at[FM:2 * FM]),
        (wg_hbm.at[FM:F], wgu_v.at[2 * FM:2 * FM + FT]),
        (wu_hbm.at[FM:F], wgu_v.at[2 * FM + FT:2 * F]), (wd_hbm, wd_v)]
    copies = [pltpu.make_async_copy(a, b, sems.at[i]) for i, (a, b) in enumerate(pairs)]

    NC = S // _TK
    neg_inf = jnp.full((8, _TQ), -jnp.inf, F32)

    def scores(t, j, c, m_run):
        t = jnp.minimum(t, NQ * _H - 1)
        f = (t % _H) * Dh
        kt = jnp.where(f % 128 + Dh > 128, NT + f // 128, f // 128)
        k = pltpu.bitcast(k_v[kt, pl.ds(c * _TK // 2, _TK // 2), :], BF16)
        q = pltpu.bitcast(qm_v[t], BF16)
        s = jnp.dot(k, q, preferred_element_type=F32)
        s_v[j % 4][jnp.minimum(t, 0), pl.ds(c * _TK, _TK), :] = s
        return jnp.maximum(m_run, jnp.max(s.reshape(_TK // 8, 8, _TQ), axis=0))

    def stage(t, j, m_cur, m_run):
        h = t % _H
        acc = jnp.zeros((_VR, _TQ), F32)
        for c in range(NC):
            if c + _LAG == NC:
                m_nxt = jnp.max(m_run, axis=0, keepdims=True)
                m_run = neg_inf
            d = 1 + (c + _LAG) // NC
            m_run = scores(t + d, j + d, (c + _LAG) % NC, m_run)
            p = jnp.exp2(s_v[j % 4][jnp.minimum(qb, 0), pl.ds(c * _TK, _TK), :] - m_cur)
            acc = acc + jnp.dot(vt_v[c, h], p.astype(BF16), preferred_element_type=F32)
        f0 = h * Dh
        rq = lax.broadcasted_iota(jnp.int32, (_VR, _TQ), 0) - f0 % 8
        hq = (rq >= 0) & (rq < Dh)
        l = jnp.max(jnp.where(hq, 0.0, acc), axis=0, keepdims=True)
        w = pl.ds(pl.multiple_of((f0 // 8) * 8, 8), _VR)
        ot_v[w, :] = jnp.where(hq, acc * (1.0 / l), ot_v[w, :])
        return m_nxt, m_run

    @pl.when(qb == 0)
    def _():
        for cp in copies[:2]:
            cp.start()
        ot_v[...] = jnp.zeros_like(ot_v)
        copies[0].wait()
        copies[2].start()

        def normalize(i):
            sl = pl.ds(pl.multiple_of(i * _TQ, _TQ), _TQ)
            return _layernorm(x_v[sl, :].astype(F32)).astype(BF16)
        xn0 = normalize(qb)
        copies[1].wait()
        copies[2].wait()
        for cp in copies[3:]:
            cp.start()

        def proj_body(i, xn):
            q = jnp.dot(xn, wqkv_v[:, 0:D], preferred_element_type=F32) * qscale
            qt = q.T
            for h in range(_H):
                blocks = [jnp.zeros((16, _TQ), F32)] * 8
                for g in range(h * Dh // 16, (h * Dh + Dh - 1) // 16 + 1):
                    r = lax.broadcasted_iota(jnp.int32, (16, _TQ), 0) + g * 16
                    blocks[g % 8] = jnp.where((r >= h * Dh) & (r < h * Dh + Dh),
                                              qt[g * 16:(g + 1) * 16], 0.0)
                qm = jnp.concatenate(blocks, axis=0).astype(BF16)
                qm_v[i * _H + h] = pltpu.bitcast(qm, jnp.uint32)
            sk = pl.ds(pl.multiple_of(i * (_TQ // 2), _TQ // 2), _TQ // 2)
            k = jnp.dot(xn, wqkv_v[:, D:2 * D], preferred_element_type=F32)
            lane = lax.broadcasted_iota(jnp.int32, (_TQ, 128), 1)
            for j in range(NT):
                kj = k[:, j * 128:(j + 1) * 128]
                k_v[j, sk, :] = pltpu.bitcast(kj.astype(BF16), jnp.uint32)
                if j + 1 < NT:
                    kn = k[:, (j + 1) * 128:(j + 2) * 128]
                    mixed = jnp.where(lane >= 64, kj, kn).astype(BF16)
                    k_v[NT + j, sk, :] = pltpu.bitcast(mixed, jnp.uint32)
            v = jnp.dot(xn, wqkv_v[:, 2 * D:3 * D], preferred_element_type=F32)
            vt = v.T
            for h in range(_H):
                r0 = h * Dh // 8 * 8
                r = lax.broadcasted_iota(jnp.int32, (_VR, _TQ), 0) + r0
                vh = jnp.where((r >= h * Dh) & (r < h * Dh + Dh), vt[r0:r0 + _VR], 1.0)
                for j in range(_TQ // _TK):
                    vt_v[i * (_TQ // _TK) + j, h] = vh[:, j * _TK:(j + 1) * _TK]
            return normalize(jnp.minimum(i + 1, NQ - 1))
        lax.fori_loop(0, NQ, proj_body, xn0)
        m_run = neg_inf
        for c in range(NC):
            m_run = scores(qb, 0, c, m_run)
        m_v[...] = jnp.max(m_run, axis=0, keepdims=True)
        m_run = neg_inf
        for c in range(_LAG):
            m_run = scores(qb + 1, 1, c, m_run)
        mr_v[...] = m_run

    def attn_body(i, m):
        t = qb * _H + _UH * i
        for j in range(_UH):
            m = stage(t + j, j, *m)
        return m
    m_v[...], mr_v[...] = lax.fori_loop(0, _H // _UH, attn_body, (m_v[...], mr_v[...]))

    @pl.when(qb == 0)
    def _():
        for cp in copies[3:]:
            cp.wait()

    TS = 256
    hs, acts = [], []
    for j in range(_TQ // TS):
        o = ot_v[:, j * TS:(j + 1) * TS].T.astype(BF16)
        xs = x_v[pl.ds(pl.multiple_of(qb * _TQ + j * TS, TS), TS), :].astype(F32)
        hs.append(xs + jnp.dot(o, wo_v[...], preferred_element_type=F32))
    for h in hs:
        hn = _layernorm(h).astype(BF16)
        gu = lax.dot_general(hn, wgu_v[...], _NT_DIMS, preferred_element_type=F32)
        g = jnp.concatenate([gu[:, :FM], gu[:, 2 * FM:2 * FM + FT]], axis=1)
        u = jnp.concatenate([gu[:, FM:2 * FM], gu[:, 2 * FM + FT:]], axis=1)
        acts.append((g * jax.nn.sigmoid(g) * u).astype(BF16))
    for j, (h, a) in enumerate(zip(hs, acts)):
        y = h + jnp.dot(a, wd_v[...], preferred_element_type=F32)
        out_ref[j * TS:(j + 1) * TS, :] = y.astype(out_ref.dtype)


@jax.jit
def pallas_sequential_preLN__mha_block__swiglu_ffn__prompt_kernel(
    A_x: jax.Array,
    A_wqkv: jax.Array,
    A_wo: jax.Array,
    B_x: jax.Array,
    B_w_gate: jax.Array,
    B_w_up: jax.Array,
    B_w_down: jax.Array,
):
    del B_x
    B, S, D = A_x.shape
    assert B == 1
    x = A_x.reshape(S, D)
    NT = D // 128
    ins = (x, A_wqkv, A_wo, B_w_gate.T, B_w_up.T, B_w_down)
    out = pl.pallas_call(
        _kernel,
        grid=(S // _TQ,),
        in_specs=[pl.BlockSpec(memory_space=pltpu.HBM)] * len(ins),
        out_specs=pl.BlockSpec((_TQ, D), lambda i: (i, 0)),
        out_shape=jax.ShapeDtypeStruct((S, D), A_x.dtype),
        scratch_shapes=[pltpu.VMEM(a.shape, a.dtype) for a in ins[:3]] + [
            pltpu.VMEM((2 * B_w_down.shape[0], D), B_w_gate.dtype),
            pltpu.VMEM(B_w_down.shape, B_w_down.dtype),
            pltpu.SemaphoreType.DMA((9,)),
            pltpu.VMEM((2 * NT - 1, S // 2, 128), jnp.uint32),
            pltpu.VMEM((S // _TQ * _H, 64, _TQ), jnp.uint32),
            pltpu.VMEM((S // _TK, _H, _VR, _TK), F32),
            [pltpu.VMEM((1, S, _TQ), F32)] * 4,
            pltpu.VMEM((1, _TQ), F32),
            pltpu.VMEM((8, _TQ), F32),
            pltpu.VMEM((D, _TQ), F32),
        ],
        compiler_params=pltpu.CompilerParams(
            dimension_semantics=("arbitrary",),
            vmem_limit_bytes=110 * 1024 * 1024),
        name="preln_mha_swiglu",
    )(*ins)
    return out.reshape(B, S, D)
```
